```python
import jax
import jax.numpy as jnp

def _softmax(x, axis=-1):
    return jax.nn.softmax(x, axis=axis)
def _gelu(x):
    return jax.nn.gelu(x, approximate=True)
def _silu(x):
    return jax.nn.silu(x)
def _sigmoid(x):
    return jax.nn.sigmoid(x)
def _layernorm(x, axis=-1, eps=1e-5):
    m = jnp.mean(x, axis=axis, keepdims=True)
    v = jnp.var(x, axis=axis, keepdims=True)
    return (x - m) / jnp.sqrt(v + eps)
def _scatter_add(tgt, idx, src, axis=0):
    return tgt.at[idx].add(src)
def _segment_sum(src, seg, n):
    return jax.ops.segment_sum(src, seg, n)
class _Rng:
    def __init__(self, key):
        self._k = key
    def _next(self):
        self._k, sub = jax.random.split(self._k)
        return sub
    def normal(self, shape):
        return jax.random.normal(self._next(), shape, dtype=jnp.bfloat16)
    def randint(self, lo, hi, shape):
        return jax.random.randint(self._next(), shape, lo, hi, dtype=jnp.int32)
    def uniform(self, shape, lo=0.0, hi=1.0):
        return jax.random.uniform(self._next(), shape, jnp.bfloat16, lo, hi)
    def permutation(self, n):
        return jax.random.permutation(self._next(), n)


kernel_name = 'standalone__gqa_softmax__near_ridge'

def setup_inputs():
    _rng = _Rng(jax.random.key(int.from_bytes(__import__("os").urandom(4), "little")))
    _w = (lambda a: (lambda t: t.astype(jnp.bfloat16) if jnp.issubdtype(t.dtype, jnp.floating) else t)(jnp.asarray(a)))
    B, Hq, Hkv, Sq, Sk, D = 16, 32, 32, 848, 512, 192
    return {
        "q": _w((lambda *s: _rng.normal(s) * 0.05)(B, Hq, Sq, D)),
        "k": _w((lambda *s: _rng.normal(s) * 0.05)(B, Hkv, Sk, D)),
        "v": _w((lambda *s: _rng.normal(s) * 0.05)(B, Hkv, Sk, D)),
    }

def reference(q, k, v):
    B, Hq, Sq, D = q.shape
    Hkv = k.shape[1]
    rep = Hq // Hkv
    k = jnp.repeat(k, rep, axis=1)
    v = jnp.repeat(v, rep, axis=1)
    scale = D ** -0.5
    scores = jnp.einsum("bhqd,bhkd->bhqk", q, k) * scale
    p = _softmax(scores, axis=-1)
    return jnp.einsum("bhqk,bhkd->bhqd", p, v)
```

```python
import math

import jax
import jax.numpy as jnp
from jax import lax
import jax.experimental.pallas as pl
import jax.experimental.pallas.tpu as pltpu

_HEADS_PER_STEP = 4


def _attn_kernel(q_ref, k_ref, v_ref, o_ref):
    d = q_ref.shape[1]
    c = (d ** -0.5) * math.log2(math.e)
    for h in range(q_ref.shape[0]):
        s_t = lax.dot_general(k_ref[h], q_ref[h], (((0,), (0,)), ((), ())),
                              preferred_element_type=jnp.float32)
        m = jnp.max(s_t, axis=0, keepdims=True)
        p = jnp.exp2((s_t - m) * c)
        l = jnp.sum(p, axis=0, keepdims=True)
        o_t = jnp.dot(v_ref[h], p.astype(jnp.bfloat16),
                      preferred_element_type=jnp.float32)
        o_ref[h] = (o_t * (1.0 / l)).astype(o_ref.dtype)


@jax.jit
def pallas_standalone__gqa_softmax__near_ridge_kernel(
    q: jax.Array,
    k: jax.Array,
    v: jax.Array,
):
    b, h, sq, d = q.shape
    sk = k.shape[2]
    assert k.shape[1] == h and v.shape[1] == h
    hb = _HEADS_PER_STEP
    q_t = jnp.swapaxes(q, 2, 3).reshape(b * h, d, sq)
    k_t = jnp.swapaxes(k, 2, 3).reshape(b * h, d, sk)
    v_t = jnp.swapaxes(v, 2, 3).reshape(b * h, d, sk)
    o_t = pl.pallas_call(
        _attn_kernel,
        grid=(b * h // hb,),
        in_specs=[
            pl.BlockSpec((hb, d, sq), lambda i: (i, 0, 0)),
            pl.BlockSpec((hb, d, sk), lambda i: (i, 0, 0)),
            pl.BlockSpec((hb, d, sk), lambda i: (i, 0, 0)),
        ],
        out_specs=pl.BlockSpec((hb, d, sq), lambda i: (i, 0, 0)),
        out_shape=jax.ShapeDtypeStruct((b * h, d, sq), q.dtype),
        compiler_params=pltpu.CompilerParams(
            dimension_semantics=("parallel",),
            vmem_limit_bytes=64 * 1024 * 1024,
        ),
        name="attn",
    )(q_t, k_t, v_t)
    return jnp.swapaxes(o_t.reshape(b, h, d, sq), 2, 3)
```

```python
import math

import jax
import jax.numpy as jnp
from jax import lax
import jax.experimental.pallas as pl
import jax.experimental.pallas.tpu as pltpu

_TQ = 256
_GROUP = 7
_N_S = 3
_N_KT = 2
_NT = (((1,), (1,)), ((), ()))
_ORDER = ("p0", "k", "p3", "q3", "p1", "q0", "q1", "q2", "p2")


def _attn_kernel(q_hbm, k_hbm, v_hbm, o_hbm,
                 q_buf, k_buf, v_buf, o_buf,
                 q_first, k_first, v_last, o_last,
                 sem, sem_edge, *scratch):
    n, d, sq = q_hbm.shape
    n_main = sq // _TQ
    n_iter = (n - 1) // _GROUP
    scratch = iter(scratch)
    kt_scr = [next(scratch) for _ in range(_N_KT)]
    s_scr = [next(scratch) for _ in range(_N_S)]
    p_scr = [[next(scratch) for _ in range(n_main + 1)] for _ in range(_GROUP)]
    r_scr = [[next(scratch) for _ in range(n_main)] for _ in range(_GROUP)]
    scale = (d ** -0.5) * math.log2(math.e)
    used = {"s": 0, "kt": 0}

    def transpose_k(k_ref, z):
        used["kt"] += 1
        kt_scr[used["kt"] % _N_KT][z[0]] = pltpu.bitcast(k_ref[...].T, jnp.uint32)

    def scores_softmax(q_ref, k_ref, slot, t, z):
        p_ref = p_scr[slot % _GROUP][t]
        if t == n_main:
            q = q_ref[:, t * _TQ:].T
            s = jnp.dot(q, k_ref[...], preferred_element_type=jnp.float32) * scale
            p = jnp.exp2(s - jnp.max(s, axis=1, keepdims=True))
            p = p * (1.0 / jnp.sum(p, axis=1, keepdims=True))
            p_ref[z[0]] = p.astype(jnp.bfloat16)
            return
        k = pltpu.bitcast(kt_scr[used["kt"] % _N_KT][z[1]], jnp.bfloat16)
        s = jnp.dot(k, q_ref[:, t * _TQ:(t + 1) * _TQ],
                    preferred_element_type=jnp.float32) * scale
        m = jnp.max(s, axis=0, keepdims=True)
        s_ref = s_scr[used["s"] % _N_S]
        used["s"] += 1
        s_ref[z[0]] = s
        p = jnp.exp2(s_ref[z[1]] - m)
        inv = 1.0 / jnp.sum(p, axis=0, keepdims=True)
        p_ref[z[0]] = p.astype(jnp.bfloat16)
        r_ref = r_scr[slot % _GROUP][t]
        r_ref[z[0]] = jnp.broadcast_to(inv, r_ref.shape[1:])

    def weighted_sum(v_ref, o_ref, slot, t, z):
        p = p_scr[slot % _GROUP][t][z[1]]
        if t == n_main:
            lo = lax.dot_general(p, v_ref[:128, :], _NT, preferred_element_type=jnp.float32)
            o_ref[:128, t * _TQ:] = lo.astype(o_ref.dtype).T
            hi = lax.dot_general(v_ref[128:, :], p, _NT, preferred_element_type=jnp.float32)
            o_ref[128:, t * _TQ:] = hi.astype(o_ref.dtype)
            return
        o = jnp.dot(v_ref[...], p, preferred_element_type=jnp.float32)
        inv = r_scr[slot % _GROUP][t][z[1]][0:1, :]
        o_ref[:, t * _TQ:(t + 1) * _TQ] = (o * inv).astype(o_ref.dtype)

    def copies_in(j, slot):
        ahead = pl.ds(j * _GROUP + 1, _GROUP)
        return (
            pltpu.make_async_copy(q_hbm.at[ahead], q_buf.at[slot], sem.at[0, slot]),
            pltpu.make_async_copy(k_hbm.at[ahead], k_buf.at[slot], sem.at[1, slot]),
            pltpu.make_async_copy(v_hbm.at[pl.ds(j * _GROUP, _GROUP)], v_buf.at[slot],
                                  sem.at[2, slot]),
        )

    def copy_out(j, slot):
        return pltpu.make_async_copy(o_buf.at[slot], o_hbm.at[pl.ds(j * _GROUP, _GROUP)],
                                     sem.at[3, slot])

    cp_k = pltpu.make_async_copy(k_hbm.at[0], k_first, sem_edge.at[0])
    cp_q = pltpu.make_async_copy(q_hbm.at[0], q_first, sem_edge.at[1])
    cp_v = pltpu.make_async_copy(v_hbm.at[n - 1], v_last, sem_edge.at[2])
    cp_o = pltpu.make_async_copy(o_last, o_hbm.at[n - 1], sem_edge.at[3])
    cp_k.start()
    cp_q.start()
    cp_k.wait()
    for cp in copies_in(0, 0):
        cp.start()
    transpose_k(k_first, (0, 0))
    cp_q.wait()
    for t in range(n_main + 1):
        scores_softmax(q_first, k_first, 0, t, (0, 0))
    cp_v.start()

    def body(j, carry):
        slot = j & 1
        z = (j >> 20, j >> 21)

        @pl.when(j + 1 < n_iter)
        def _():
            for cp in copies_in(j + 1, 1 - slot):
                cp.start()

        @pl.when(j >= 2)
        def _():
            copy_out(j - 2, slot).wait()

        for cp in copies_in(j, slot):
            cp.wait()
        for g in range(_GROUP):
            for op in _ORDER:
                if op == "k":
                    transpose_k(k_buf.at[slot, g], z)
                elif op[0] == "p":
                    weighted_sum(v_buf.at[slot, g], o_buf.at[slot, g], g, int(op[1]), z)
                else:
                    scores_softmax(q_buf.at[slot, g], k_buf.at[slot, g], g + 1, int(op[1]), z)
        copy_out(j, slot).start()
        return carry

    lax.fori_loop(0, n_iter, body, 0)

    cp_v.wait()
    for t in range(n_main + 1):
        weighted_sum(v_last, o_last, 0, t, (0, 0))
    cp_o.start()
    copy_out(n_iter - 2, n_iter % 2).wait()
    copy_out(n_iter - 1, (n_iter - 1) % 2).wait()
    cp_o.wait()


@jax.jit
def pallas_standalone__gqa_softmax__near_ridge_kernel(
    q: jax.Array,
    k: jax.Array,
    v: jax.Array,
):
    b, h, sq, d = q.shape
    sk = k.shape[2]
    n = b * h
    assert k.shape[1] == h and v.shape[1] == h
    assert (n - 1) % _GROUP == 0 and n - 1 >= 2 * _GROUP and sq // _TQ == 3
    q_t = jnp.swapaxes(q, 2, 3).reshape(n, d, sq)
    k_t = jnp.swapaxes(k, 2, 3).reshape(n, d, sk)
    v_t = jnp.swapaxes(v, 2, 3).reshape(n, d, sk)

    bf16, f32 = jnp.bfloat16, jnp.float32
    n_main = sq // _TQ
    scratch = [
        pltpu.VMEM((2, _GROUP, d, sq), bf16),
        pltpu.VMEM((2, _GROUP, d, sk), bf16),
        pltpu.VMEM((2, _GROUP, d, sk), bf16),
        pltpu.VMEM((2, _GROUP, d, sq), bf16),
        pltpu.VMEM((d, sq), bf16),
        pltpu.VMEM((d, sk), bf16),
        pltpu.VMEM((d, sk), bf16),
        pltpu.VMEM((d, sq), bf16),
        pltpu.SemaphoreType.DMA((4, 2)),
        pltpu.SemaphoreType.DMA((4,)),
    ]
    scratch += [pltpu.VMEM((1, sk // 2, d), jnp.uint32)] * _N_KT
    scratch += [pltpu.VMEM((1, sk, _TQ), f32)] * _N_S
    scratch += ([pltpu.VMEM((1, sk, _TQ), bf16)] * n_main
                + [pltpu.VMEM((1, sq % _TQ, sk), bf16)]) * _GROUP
    scratch += [pltpu.VMEM((1, 8, _TQ), f32)] * (n_main * _GROUP)

    o_t = pl.pallas_call(
        _attn_kernel,
        in_specs=[pl.BlockSpec(memory_space=pl.ANY)] * 3,
        out_specs=pl.BlockSpec(memory_space=pl.ANY),
        out_shape=jax.ShapeDtypeStruct((n, d, sq), q.dtype),
        scratch_shapes=scratch,
        compiler_params=pltpu.CompilerParams(
            vmem_limit_bytes=100 * 1024 * 1024,
            disable_bounds_checks=True,
            flags={"XLA_TPU_FORCE_LP_LLO_SCHEDULER": True},
        ),
        name="attn",
    )(q_t, k_t, v_t)
    return jnp.swapaxes(o_t.reshape(b, h, d, sq), 2, 3)
```

```python
import math

import jax
import jax.numpy as jnp
from jax import lax
import jax.experimental.pallas as pl
import jax.experimental.pallas.tpu as pltpu

_TQ = 256
_GROUP = 10
_RAMP_IN = (2, 5)
_RAMP_OUT = (3, 1)
_N_S = 3
_N_KT = 2
_NT = (((1,), (1,)), ((), ()))
_ORDER = ("p3", "k", "p0", "q3", "p1", "q0", "q1", "q2", "p2")


def _attn_kernel(q_hbm, k_hbm, v_hbm, o_hbm,
                 q_buf, k_buf, v_buf, o_buf,
                 q_first, k_first, v_last, o_last,
                 sem_main, sem_end, sem_ramp, *scratch):
    n, d, sq = q_hbm.shape
    n_main = sq // _TQ
    ramps = _RAMP_IN + _RAMP_OUT
    n_in = len(_RAMP_IN)
    h_loop = sum(_RAMP_IN)
    n_iter = (n - 1 - sum(ramps)) // _GROUP
    ramp_start = [sum(ramps[:e]) + (n_iter * _GROUP if e >= n_in else 0)
                  for e in range(len(ramps))]
    scratch = iter(scratch)
    kt_scr = [next(scratch) for _ in range(_N_KT)]
    s_scr = [next(scratch) for _ in range(_N_S)]
    p_scr = [[next(scratch) for _ in range(n_main + 1)] for _ in range(_GROUP)]
    r_scr = [[next(scratch) for _ in range(n_main)] for _ in range(_GROUP)]
    ramp_buf = [[next(scratch) for _ in range(4)] for _ in ramps]
    scale = (d ** -0.5) * math.log2(math.e)
    used = {"s": 0, "kt": 0}

    def transpose_k(k_ref, z):
        used["kt"] += 1
        kt_scr[used["kt"] % _N_KT][z[0]] = pltpu.bitcast(k_ref[...].T, jnp.uint32)

    def scores_softmax(q_ref, k_ref, slot, t, z):
        p_ref = p_scr[slot % _GROUP][t]
        if t == n_main:
            q = q_ref[:, t * _TQ:].T
            s = jnp.dot(q, k_ref[...], preferred_element_type=jnp.float32) * scale
            p = jnp.exp2(s - jnp.max(s, axis=1, keepdims=True))
            p = p * (1.0 / jnp.sum(p, axis=1, keepdims=True))
            p_ref[z[0]] = p.astype(jnp.bfloat16)
            return
        k = pltpu.bitcast(kt_scr[used["kt"] % _N_KT][z[1]], jnp.bfloat16)
        s = jnp.dot(k, q_ref[:, t * _TQ:(t + 1) * _TQ],
                    preferred_element_type=jnp.float32) * scale
        m = jnp.max(s, axis=0, keepdims=True)
        s_ref = s_scr[used["s"] % _N_S]
        used["s"] += 1
        s_ref[z[0]] = s
        p = jnp.exp2(s_ref[z[1]] - m)
        inv = 1.0 / jnp.sum(p, axis=0, keepdims=True)
        p_ref[z[0]] = p.astype(jnp.bfloat16)
        r_ref = r_scr[slot % _GROUP][t]
        r_ref[z[0]] = jnp.broadcast_to(inv, r_ref.shape[1:])

    def weighted_sum(v_ref, o_ref, slot, t, z):
        p = p_scr[slot % _GROUP][t][z[1]]
        if t == n_main:
            lo = lax.dot_general(p, v_ref[:128, :], _NT, preferred_element_type=jnp.float32)
            o_ref[:128, t * _TQ:] = lo.astype(o_ref.dtype).T
            hi = lax.dot_general(v_ref[128:, :], p, _NT, preferred_element_type=jnp.float32)
            o_ref[128:, t * _TQ:] = hi.astype(o_ref.dtype)
            return
        o = jnp.dot(v_ref[...], p, preferred_element_type=jnp.float32)
        inv = r_scr[slot % _GROUP][t][z[1]][0:1, :]
        o_ref[:, t * _TQ:(t + 1) * _TQ] = (o * inv).astype(o_ref.dtype)

    def run_group(bufs, slot0, z):
        q_ref, k_ref, v_ref, o_ref = bufs
        for g in range(q_ref.shape[0]):
            for op in _ORDER:
                if op == "k":
                    transpose_k(k_ref.at[g], z)
                elif op[0] == "p":
                    weighted_sum(v_ref.at[g], o_ref.at[g], slot0 + g, int(op[1]), z)
                else:
                    scores_softmax(q_ref.at[g], k_ref.at[g], slot0 + g + 1, int(op[1]), z)

    def main_group(j, slot):
        return (h_loop + j * _GROUP,
                [buf.at[slot] for buf in (q_buf, k_buf, v_buf, o_buf)],
                [sem_main.at[i, slot] for i in range(4)])

    def ramp_group(e):
        return ramp_start[e], ramp_buf[e], [sem_ramp.at[e, i] for i in range(4)]

    def loads(group):
        h, bufs, sems = group
        size = bufs[0].shape[0]
        return [pltpu.make_async_copy(src.at[pl.ds(h + ahead, size)], bufs[i], sems[i])
                for i, (src, ahead) in enumerate(((q_hbm, 1), (k_hbm, 1), (v_hbm, 0)))]

    def store(group):
        h, bufs, sems = group
        return pltpu.make_async_copy(bufs[3], o_hbm.at[pl.ds(h, bufs[3].shape[0])], sems[3])

    def start_loads(group):
        for cp in loads(group):
            cp.start()

    def wait_loads(group):
        for cp in loads(group):
            cp.wait()

    cp_k = pltpu.make_async_copy(k_hbm.at[0], k_first, sem_end.at[0])
    cp_q = pltpu.make_async_copy(q_hbm.at[0], q_first, sem_end.at[1])
    cp_v = pltpu.make_async_copy(v_hbm.at[n - 1], v_last, sem_end.at[2])
    cp_o = pltpu.make_async_copy(o_last, o_hbm.at[n - 1], sem_end.at[3])

    upcoming = [ramp_group(e) for e in range(n_in)] + [main_group(0, 0)]
    cp_k.start()
    cp_q.start()
    cp_k.wait()
    start_loads(upcoming[0])
    one = lax.fori_loop(0, 2, lambda i, c: c + i, 0)
    z_edge = (one >> 20, one >> 21)
    transpose_k(k_first, z_edge)
    cp_q.wait()
    start_loads(upcoming[1])
    for t in range(n_main + 1):
        scores_softmax(q_first, k_first, -h_loop, t, z_edge)
    for e in range(n_in):
        wait_loads(upcoming[e])
        if e + 2 < len(upcoming):
            start_loads(upcoming[e + 2])
        run_group(ramp_buf[e], ramp_start[e] - h_loop, z_edge)
    wait_loads(main_group(0, 0))
    start_loads(main_group(1, 1))

    def body(j, carry):
        slot = j & 1
        cur = main_group(j, slot)
        run_group(cur[1], 0, (j >> 20, j >> 21))
        store(cur).start()

        @pl.when(j + 2 < n_iter)
        def _():
            start_loads(main_group(j + 2, slot))

        @pl.when(j == 1)
        def _():
            for e in range(n_in):
                store(ramp_group(e)).start()

        @pl.when(j + 2 == n_iter)
        def _():
            cp_v.start()
            for e in range(n_in, len(ramps)):
                start_loads(ramp_group(e))

        @pl.when(j + 1 < n_iter)
        def _():
            wait_loads(main_group(j + 1, 1 - slot))

        @pl.when(j >= 1)
        def _():
            store(main_group(j - 1, 1 - slot)).wait()

        return carry

    lax.fori_loop(0, n_iter, body, 0)

    for e in range(n_in, len(ramps)):
        wait_loads(ramp_group(e))
        run_group(ramp_buf[e], ramp_start[e] - h_loop, z_edge)
        store(ramp_group(e)).start()
    cp_v.wait()
    for t in range(n_main + 1):
        weighted_sum(v_last, o_last, n - 1 - h_loop, t, z_edge)
    cp_o.start()
    for e in range(len(ramps)):
        store(ramp_group(e)).wait()
    store(main_group(n_iter - 1, (n_iter - 1) % 2)).wait()
    cp_o.wait()


@jax.jit
def pallas_standalone__gqa_softmax__near_ridge_kernel(
    q: jax.Array,
    k: jax.Array,
    v: jax.Array,
):
    b, h, sq, d = q.shape
    sk = k.shape[2]
    n = b * h
    in_loop = n - 1 - sum(_RAMP_IN) - sum(_RAMP_OUT)
    assert k.shape[1] == h and v.shape[1] == h and sq // _TQ == 3
    assert in_loop % _GROUP == 0 and in_loop >= 2 * _GROUP
    q_t = jnp.swapaxes(q, 2, 3).reshape(n, d, sq)
    k_t = jnp.swapaxes(k, 2, 3).reshape(n, d, sk)
    v_t = jnp.swapaxes(v, 2, 3).reshape(n, d, sk)

    bf16, f32 = jnp.bfloat16, jnp.float32
    n_main = sq // _TQ

    def qkvo(*lead):
        return [pltpu.VMEM((*lead, d, s), bf16) for s in (sq, sk, sk, sq)]

    scratch = qkvo(2, _GROUP) + qkvo() + [
        pltpu.SemaphoreType.DMA((4, 2)),
        pltpu.SemaphoreType.DMA((4,)),
        pltpu.SemaphoreType.DMA((len(_RAMP_IN) + len(_RAMP_OUT), 4)),
    ]
    scratch += [pltpu.VMEM((1, sk // 2, d), jnp.uint32)] * _N_KT
    scratch += [pltpu.VMEM((1, sk, _TQ), f32)] * _N_S
    scratch += ([pltpu.VMEM((1, sk, _TQ), bf16)] * n_main
                + [pltpu.VMEM((1, sq % _TQ, sk), bf16)]) * _GROUP
    scratch += [pltpu.VMEM((1, 8, _TQ), f32)] * (n_main * _GROUP)
    for size in _RAMP_IN + _RAMP_OUT:
        scratch += qkvo(size)

    o_t = pl.pallas_call(
        _attn_kernel,
        in_specs=[pl.BlockSpec(memory_space=pl.ANY)] * 3,
        out_specs=pl.BlockSpec(memory_space=pl.ANY),
        out_shape=jax.ShapeDtypeStruct((n, d, sq), q.dtype),
        scratch_shapes=scratch,
        compiler_params=pltpu.CompilerParams(
            vmem_limit_bytes=100 * 1024 * 1024,
            disable_bounds_checks=True,
            flags={"XLA_TPU_FORCE_LP_LLO_SCHEDULER": True},
        ),
        name="attn",
    )(q_t, k_t, v_t)
    return jnp.swapaxes(o_t.reshape(b, h, d, sq), 2, 3)
```
